```python
import os as _os
_os.environ.setdefault("JAX_PLATFORMS", "cpu")
import jax
import jax.numpy as jnp

def _softmax(x, axis=-1):
    return jax.nn.softmax(x, axis=axis)
def _gelu(x):
    return jax.nn.gelu(x, approximate=True)
def _silu(x):
    return jax.nn.silu(x)
def _sigmoid(x):
    return jax.nn.sigmoid(x)
def _layernorm(x, axis=-1, eps=1e-5):
    m = jnp.mean(x, axis=axis, keepdims=True)
    v = jnp.var(x, axis=axis, keepdims=True)
    return (x - m) / jnp.sqrt(v + eps)
def _scatter_add(tgt, idx, src, axis=0):
    return tgt.at[idx].add(src)
def _segment_sum(src, seg, n):
    return jax.ops.segment_sum(src, seg, n)
class _Rng:
    def __init__(self, key):
        self._k = key
    def _next(self):
        self._k, sub = jax.random.split(self._k)
        return sub
    def normal(self, shape):
        return jax.random.normal(self._next(), shape, dtype=jnp.bfloat16)
    def randint(self, lo, hi, shape):
        return jax.random.randint(self._next(), shape, lo, hi, dtype=jnp.int32)
    def uniform(self, shape, lo=0.0, hi=1.0):
        return jax.random.uniform(self._next(), shape, jnp.bfloat16, lo, hi)
    def permutation(self, n):
        return jax.random.permutation(self._next(), n)


kernel_name = 'concat_heads__ssm_conv_s4__linear_attn_block__prompt'

def setup_inputs():
    _rng = _Rng(jax.random.key(int.from_bytes(__import__("os").urandom(4), "little")))
    _w = (lambda a: (lambda t: t.astype(jnp.bfloat16) if jnp.issubdtype(t.dtype, jnp.floating) else t)(jnp.asarray(a)))
    def _A_setup():
        B, L, D, N = 1, 2048, 512, 128
        A_re = -jnp.exp((lambda *s: _rng.normal(s) * 0.1)(D, N))
        A_im = jnp.pi * (lambda *s: _rng.normal(s) * 0.1)(D, N)
        B_re = (lambda *s: _rng.normal(s) * 0.1)(D, N)
        B_im = (lambda *s: _rng.normal(s) * 0.1)(D, N)
        C_re = (lambda *s: _rng.normal(s) * 0.1)(D, N)
        C_im = (lambda *s: _rng.normal(s) * 0.1)(D, N)
        log_dt = (lambda *s: _rng.normal(s) * 0.1)(D) * 0.5 - 4.0
        Dskip = (lambda *s: _rng.normal(s) * 0.05)(D)
        return {
            "u": _w((lambda *s: _rng.normal(s) * 0.05)(B, L, D)),
            "A_re": _w(A_re),
            "A_im": _w(A_im),
            "B_re": _w(B_re),
            "B_im": _w(B_im),
            "C_re": _w(C_re),
            "C_im": _w(C_im),
            "log_dt": _w(log_dt),
            "Dskip": _w(Dskip),
        }
    _A_in = _A_setup()

    def _B_setup():
        B, S, D = 1, 2048, 512
        return {
            "x": _w((lambda *s: _rng.normal(s) * 0.05)(B, S, D)),
            "wqkv": _w((lambda *s: _rng.normal(s) * 0.4)(D, 3 * D)),
            "wo": _w((lambda *s: _rng.normal(s) * 0.05)(D, D)),
        }
    _B_in = _B_setup()

    return {
        "A_u": _A_in["u"],
        "A_A_re": _A_in["A_re"],
        "A_A_im": _A_in["A_im"],
        "A_B_re": _A_in["B_re"],
        "A_B_im": _A_in["B_im"],
        "A_C_re": _A_in["C_re"],
        "A_C_im": _A_in["C_im"],
        "A_log_dt": _A_in["log_dt"],
        "A_Dskip": _A_in["Dskip"],
        "B_x": _B_in["x"],
        "B_wqkv": _B_in["wqkv"],
        "B_wo": _B_in["wo"],
    }

def reference(A_u, A_A_re, A_A_im, A_B_re, A_B_im, A_C_re, A_C_im, A_log_dt, A_Dskip, B_x, B_wqkv, B_wo):
    def _A_ref(u, A_re, A_im, B_re, B_im, C_re, C_im, log_dt, Dskip):
        Bsz, L, D = u.shape
        dt = jnp.exp(log_dt)[:, None]
        A = A_re + 1j * A_im
        Bc = B_re + 1j * B_im
        Cc = C_re + 1j * C_im
        logdA = dt * A
        dB = dt * Bc
        l = (lambda x, dt: x.astype(dt))(jnp.arange(L), A_re.dtype)
        P = jnp.exp(logdA[:, :, None] * l[None, None, :])
        K = jnp.einsum("dn,dnl,dn->dl", Cc, P, dB).real
        L2 = 2 * L
        Kp = jnp.pad(K, ((0, 0), (0, L)))
        up = (lambda x, *d: x.transpose(*d))(u, 0, 2, 1)
        up = jnp.pad(up, ((0, 0), (0, 0), (0, L)))
        Kf = (lambda x, axes=(-2,-1): jnp.fft.rfft2(x.astype(jnp.float32), axes=axes))(Kp[:, None, :], axes=(-2, -1))
        Uf = (lambda x, axes=(-2,-1): jnp.fft.rfft2(x.astype(jnp.float32), axes=axes))(up[:, :, None, :], axes=(-2, -1))
        Yf = Uf * Kf[None, :, :, :]
        y = (lambda x, s, axes=(-2,-1): jnp.fft.irfft2(x, s=s, axes=axes).astype(jnp.bfloat16))(Yf, (1, L2), axes=(-2, -1))[:, :, 0, :L]
        y = (lambda x, *d: x.transpose(*d))(y, 0, 2, 1) + u * Dskip[None, None, :]
        return y

    def _B_ref(x, wqkv, wo):
        B, S, D = x.shape
        H = 32; Dh = D // H
        qkv = (lambda x, *d: x.transpose(*d))((x @ wqkv).reshape(B, S, 3, H, Dh), 2, 0, 3, 1, 4)
        q, k, v = qkv[0], qkv[1], qkv[2]
        phi = lambda t: jnp.where(t > 0, t + 1, jnp.exp(t)) + 1e-6
        pq, pk = phi(q), phi(k)
        kv = jnp.einsum("bhsd,bhse->bhde", pk, v)
        z = jnp.einsum("bhsd->bhd", pk)
        num = jnp.einsum("bhqd,bhde->bhqe", pq, kv)
        den = jnp.einsum("bhqd,bhd->bhq", pq, z)[..., None] + 1e-6
        o = num / den
        return (lambda x, *d: x.transpose(*d))(o, 0, 2, 1, 3).reshape(B, S, D) @ wo

    a = _A_ref(A_u, A_A_re, A_A_im, A_B_re, A_B_im, A_C_re, A_C_im, A_log_dt, A_Dskip)
    b = _B_ref(B_x, B_wqkv, B_wo)
    return jnp.concatenate([a, b], axis=-1)
```

```python
import numpy as np
import jax
import jax.numpy as jnp
import jax.experimental.pallas as pl
import jax.experimental.pallas.tpu as pltpu

BF, F32 = jnp.bfloat16, jnp.float32


def _consts():
    k1 = np.arange(128) + 0.5
    w = np.exp(-2j * np.pi * np.outer(k1, np.arange(128)) / 256)
    F1 = np.concatenate([w.real, w.imag], 0)
    Fi = F1.T * (2.0 / 4096)
    G = np.zeros((32, 128, 128))
    t2 = np.arange(16)
    for k in range(128):
        g = np.exp(-2j * np.pi * (np.outer(np.arange(16), t2) / 16 + t2[None] * k1[k] / 4096))
        b = np.block([[g.real, -g.imag], [g.imag, g.real]])
        j = k % 4 * 32
        G[k // 4, j:j + 32, j:j + 32] = b
    return F1, Fi, G, np.transpose(G, (0, 2, 1))


def _rho(t2, sp):
    q, r = divmod(t2, sp)
    if 2 * r > sp or (2 * r == sp and q % 2):
        q += 1
    return q * sp


def _cm(a, b):
    return a[0] * b[0] - a[1] * b[1], a[0] * b[1] + a[1] * b[0]


def _dot(a, b):
    return jnp.dot(a.astype(BF), b.astype(BF), preferred_element_type=F32)


def _dnt(a, b):
    return jax.lax.dot_general(a.astype(BF), b.astype(BF), (((1,), (1,)), ((), ())),
                               preferred_element_type=F32)


def _kern(u, are, aim, bre, bim, cre, cim, ldt, dsk, x, wqkv, wo, F1, Fi, G, GT,
          o, pw, kx, s1, s2, uf, qs):
    xv = x[...]
    def phi(t):
        return jnp.where(t > 0, t + 1, jnp.exp(t)) + 1e-6
    ri = jax.lax.broadcasted_iota(jnp.int32, (128, 128), 0) // 16
    ci = jax.lax.broadcasted_iota(jnp.int32, (128, 128), 1) // 16
    m = ri == ci
    ones = m.astype(BF)
    for j in range(4):
        sl = slice(j * 128, j * 128 + 128)
        pk = phi(_dot(xv, wqkv[:, 512 + j * 128:640 + j * 128])).astype(BF)
        v = _dot(xv, wqkv[:, 1024 + j * 128:1152 + j * 128])
        kv = jax.lax.dot_general(pk, v.astype(BF), (((0,), (0,)), ((), ())),
                                 preferred_element_type=F32)
        z = jnp.sum(pk.astype(F32), 0, keepdims=True)
        pq = phi(_dot(xv, wqkv[:, sl]))
        num = _dot(pq, jnp.where(m, kv, 0.0))
        den = _dot(pq * z, ones) + 1e-6
        qs[:, sl] = (num / den).astype(BF)
    o[:, 512:] = _dot(qs[...], wo[...]).astype(BF)

    dt = jnp.exp(ldt[...].astype(F32)).astype(BF).astype(F32)
    ar = are[...].astype(F32) * dt
    ai = aim[...].astype(F32) * dt
    c = _cm((cre[...].astype(F32), cim[...].astype(F32)),
            (bre[...].astype(F32) * dt, bim[...].astype(F32) * dt))
    pw[16], pw[17] = c
    for i, p in enumerate((1., 16.)):
        e = jnp.exp(ar * p)
        z = (e * jnp.cos(ai * p), e * jnp.sin(ai * p))
        for b in range(4):
            pw[8 * i + 2 * b], pw[8 * i + 2 * b + 1] = z
            z = _cm(z, z)
    row = jax.lax.broadcasted_iota(jnp.int32, (8, 128), 0)

    def chan(d, _):
        def ld(i):
            return (jnp.broadcast_to(pw[2 * i, pl.ds(d, 1), :], (8, 128)),
                    jnp.broadcast_to(pw[2 * i + 1, pl.ds(d, 1), :], (8, 128)))
        def base(i0, init):
            r = init
            for b in range(3):
                p = ld(i0 + b)
                on = (row >> b) & 1 == 1
                p = (jnp.where(on, p[0], 1.0), jnp.where(on, p[1], 0.0))
                r = p if r is None else _cm(r, p)
            return r
        q0 = base(0, ld(8))
        q1 = _cm(q0, ld(3))
        q2 = _cm(ld(8), ld(4))
        Q = jnp.concatenate([jnp.concatenate([q[0], -q[1]], 1) for q in (q0, q1, q2)], 0)
        p = base(4, None)
        st = ld(7)
        ps = [p]
        for _i in range(15):
            p = _cm(p, st)
            ps.append(p)
        P = jnp.concatenate([jnp.concatenate(list(q), 1) for q in ps], 0)
        kx[pl.ds(pl.multiple_of(d * 24, 8), 24), :] = _dnt(Q, P)
        return 0
    jax.lax.fori_loop(0, 512, chan, 0, unroll=4)

    lane = jax.lax.broadcasted_iota(jnp.int32, (128, 128), 1)

    def stage2(g, s, row0):
        return jnp.concatenate(
            [s[pl.ds(row0 + r * 128 + g * 4 + j, 16, stride=256), :]
             for j in range(4) for r in range(2)], 0)

    for c in range(4):
        cs = slice(c * 128, c * 128 + 128)
        uf[...] = u[:, cs].astype(F32)
        for t2 in range(16):
            kt = kx[pl.ds(c * 3072 + t2, 128, stride=24), :]
            for sp, lo in ((2, 16), (4, 32), (8, 64)):
                r = _rho(t2, sp)
                if r != t2:
                    kt = jnp.where(lane >= lo, kx[pl.ds(c * 3072 + r, 128, stride=24), :], kt)
            s1[t2 * 256:(t2 + 1) * 256, :] = _dnt(F1[...], kt)
            s2[t2 * 256:(t2 + 1) * 256, :] = _dot(F1[...], uf[pl.ds(t2, 128, stride=16), :])

        def grp(g, _):
            a = _dot(G[g], stage2(g, s1, 0))
            b = _dot(G[g], stage2(g, s2, 0))
            ys = []
            for j in range(4):
                q = j * 32
                ys += list(_cm((a[q:q + 16], a[q + 16:q + 32]), (b[q:q + 16], b[q + 16:q + 32])))
            y = _dot(GT[g], jnp.concatenate(ys, 0))
            for j in range(4):
                for r in range(2):
                    q = j * 32 + r * 16
                    s2[pl.ds(r * 128 + g * 4 + j, 16, stride=256), :] = y[q:q + 16]
            return 0
        jax.lax.fori_loop(0, 32, grp, 0, unroll=2)

        for t2 in range(16):
            s1[pl.ds(t2, 128, stride=16), :] = _dot(Fi[...], s2[t2 * 256:(t2 + 1) * 256, :])
        y = s1[0:2048, :].astype(BF).astype(F32)
        o[:, cs] = (y + (u[:, cs] * dsk[:, cs]).astype(F32)).astype(BF)


@jax.jit
def pallas_concat_heads__ssm_conv_s4__linear_attn_block__prompt_kernel(
        A_u, A_A_re, A_A_im, A_B_re, A_B_im, A_C_re, A_C_im, A_log_dt, A_Dskip,
        B_x, B_wqkv, B_wo):
    cs = [jnp.asarray(c, dtype=BF) for c in _consts()]
    out = pl.pallas_call(
        _kern,
        out_shape=jax.ShapeDtypeStruct((2048, 1024), BF),
        scratch_shapes=[pltpu.VMEM((18, 512, 128), F32), pltpu.VMEM((512 * 24, 128), F32),
                        pltpu.VMEM((4096, 128), F32), pltpu.VMEM((4096, 128), F32),
                        pltpu.VMEM((2048, 128), F32), pltpu.VMEM((2048, 512), BF)],
        compiler_params=pltpu.CompilerParams(vmem_limit_bytes=100 * 1024 * 1024),
    )(A_u[0], A_A_re, A_A_im, A_B_re, A_B_im, A_C_re, A_C_im, A_log_dt.reshape(512, 1),
      A_Dskip.reshape(1, 512), B_x[0], B_wqkv, B_wo, *cs)
    return out[None]
```
